```python
import os as _os
_os.environ.setdefault("JAX_PLATFORMS", "cpu")
import jax
import jax.numpy as jnp

def _softmax(x, axis=-1):
    return jax.nn.softmax(x, axis=axis)
def _gelu(x):
    return jax.nn.gelu(x, approximate=True)
def _silu(x):
    return jax.nn.silu(x)
def _sigmoid(x):
    return jax.nn.sigmoid(x)
def _layernorm(x, axis=-1, eps=1e-5):
    m = jnp.mean(x, axis=axis, keepdims=True)
    v = jnp.var(x, axis=axis, keepdims=True)
    return (x - m) / jnp.sqrt(v + eps)
def _scatter_add(tgt, idx, src, axis=0):
    return tgt.at[idx].add(src)
def _segment_sum(src, seg, n):
    return jax.ops.segment_sum(src, seg, n)
class _Rng:
    def __init__(self, key):
        self._k = key
    def _next(self):
        self._k, sub = jax.random.split(self._k)
        return sub
    def normal(self, shape):
        return jax.random.normal(self._next(), shape, dtype=jnp.bfloat16)
    def randint(self, lo, hi, shape):
        return jax.random.randint(self._next(), shape, lo, hi, dtype=jnp.int32)
    def uniform(self, shape, lo=0.0, hi=1.0):
        return jax.random.uniform(self._next(), shape, jnp.bfloat16, lo, hi)
    def permutation(self, n):
        return jax.random.permutation(self._next(), n)


kernel_name = 'standalone__gqa_block_cached__near_ridge'

def setup_inputs():
    _rng = _Rng(jax.random.key(int.from_bytes(__import__("os").urandom(4), "little")))
    _w = (lambda a: (lambda t: t.astype(jnp.bfloat16) if jnp.issubdtype(t.dtype, jnp.floating) else t)(jnp.asarray(a)))
    B, Sq, D = 8, 80, 512
    Hq, Hkv, Sk, Dh = 32, 8, 2048, 128
    assert Hq % Hkv == 0, (Hq, Hkv)
    return {
        "x": _w((lambda *s: _rng.normal(s) * 0.8)(B, Sq, D)),
        "k_cache": _w((lambda *s: _rng.normal(s) * 0.8)(B, Hkv, Sk, Dh)),
        "v_cache": _w((lambda *s: _rng.normal(s) * 0.05)(B, Hkv, Sk, Dh)),
        "wq": _w((lambda *s: _rng.normal(s) * 0.8)(D, Hq * Dh) * (D ** -0.5)),
        "wo": _w((lambda *s: _rng.normal(s) * 0.05)(Hq * Dh, D) * ((Hq * Dh) ** -0.5)),
    }

def reference(x, k_cache, v_cache, wq, wo):
    B, Sq, D = x.shape
    Hq, Dh = 32, 128
    Hkv = k_cache.shape[1]
    rep = Hq // Hkv
    q = (lambda x, *d: x.transpose(*d))((x @ wq).reshape(B, Sq, Hq, Dh), 0, 2, 1, 3)
    k = jnp.repeat(k_cache, rep, axis=1)
    v = jnp.repeat(v_cache, rep, axis=1)
    scores = jnp.einsum("bhqd,bhkd->bhqk", q, k) * (Dh ** -0.5)
    p = _softmax(scores, axis=-1)
    o = jnp.einsum("bhqk,bhkd->bhqd", p, v)
    return (lambda x, *d: x.transpose(*d))(o, 0, 2, 1, 3).reshape(B, Sq, Hq * Dh) @ wo
```

```python
import functools
import math

import jax
import jax.numpy as jnp
import jax.experimental.pallas as pl
import jax.experimental.pallas.tpu as pltpu

HQ = 32
DH = 128


def _kernel(x_ref, k_ref, v_ref, wq_ref, wo_ref, out_ref, q_scr, o_scr, acc_scr,
            *, B, Sq, rep, Hkv, scale):
    g = pl.program_id(0)
    b = pl.program_id(1)

    @pl.when(b == 0)
    def _():
        q_all = jnp.dot(x_ref[...], wq_ref[...], preferred_element_type=jnp.float32)
        q_all = (q_all * scale).astype(jnp.bfloat16)
        for bb in range(B):
            for r in range(rep):
                q_scr[bb, r * Sq:(r + 1) * Sq, :] = q_all[bb * Sq:(bb + 1) * Sq, r * DH:(r + 1) * DH]

    q = q_scr[b]
    s = jax.lax.dot_general(q, k_ref[...], (((1,), (1,)), ((), ())),
                            preferred_element_type=jnp.float32)
    m = jnp.max(s, axis=-1, keepdims=True)
    p = jnp.exp2(s - m)
    l = jnp.sum(p, axis=-1, keepdims=True)
    o = jnp.dot(p.astype(jnp.bfloat16), v_ref[...], preferred_element_type=jnp.float32)
    o = (o / l).astype(jnp.bfloat16)
    for r in range(rep):
        o_scr[b, :, r * DH:(r + 1) * DH] = o[r * Sq:(r + 1) * Sq, :]

    @pl.when(b == B - 1)
    def _():
        o_all = o_scr[...].reshape(B * Sq, rep * DH)
        contrib = jnp.dot(o_all, wo_ref[...], preferred_element_type=jnp.float32)

        @pl.when(g == 0)
        def _():
            acc_scr[...] = contrib

        @pl.when(jnp.logical_and(g > 0, g < Hkv - 1))
        def _():
            acc_scr[...] += contrib

        @pl.when(g == Hkv - 1)
        def _():
            out_ref[...] = (acc_scr[...] + contrib).astype(out_ref.dtype)


@jax.jit
def pallas_standalone__gqa_block_cached__near_ridge_kernel(x, k_cache, v_cache, wq, wo):
    B, Sq, D = x.shape
    _, Hkv, Sk, Dh = k_cache.shape
    rep = HQ // Hkv
    scale = (Dh ** -0.5) * math.log2(math.e)
    x2 = x.reshape(B * Sq, D)
    kern = functools.partial(_kernel, B=B, Sq=Sq, rep=rep, Hkv=Hkv, scale=scale)
    out = pl.pallas_call(
        kern,
        grid=(Hkv, B),
        in_specs=[
            pl.BlockSpec((B * Sq, D), lambda g, b: (0, 0)),
            pl.BlockSpec((None, None, Sk, Dh), lambda g, b: (b, g, 0, 0)),
            pl.BlockSpec((None, None, Sk, Dh), lambda g, b: (b, g, 0, 0)),
            pl.BlockSpec((D, rep * Dh), lambda g, b: (0, g)),
            pl.BlockSpec((rep * Dh, D), lambda g, b: (g, 0)),
        ],
        out_specs=pl.BlockSpec((B * Sq, D), lambda g, b: (0, 0)),
        out_shape=jax.ShapeDtypeStruct((B * Sq, D), x.dtype),
        scratch_shapes=[
            pltpu.VMEM((B, rep * Sq, Dh), jnp.bfloat16),
            pltpu.VMEM((B, Sq, rep * Dh), jnp.bfloat16),
            pltpu.VMEM((B * Sq, D), jnp.float32),
        ],
        compiler_params=pltpu.CompilerParams(
            dimension_semantics=("arbitrary", "arbitrary"),
            vmem_limit_bytes=64 * 1024 * 1024,
        ),
    )(x2, k_cache, v_cache, wq, wo)
    return out.reshape(B, Sq, D)
```

```python
import functools
import math

import jax
import jax.numpy as jnp
import jax.experimental.pallas as pl
import jax.experimental.pallas.tpu as pltpu

HQ = 32
DH = 128
NB = 6
QW = (1, 2, 5)
NWO = 8
QSPLIT = 1024
OSPLIT = 4
FING = 2

_NT = (((1,), (1,)), ((), ()))


def _kernel(x_hbm, k_hbm, v_hbm, wq_hbm, wo_hbm, out_hbm,
            x_scr, wq_scr, wo_scr, k_buf, v_buf, qo_scr, st_scr, out_scr,
            x_sem, wq_sem, wo_sem, k_sem, v_sem, out_sem,
            *, B, Sq, Sk, D, rep, Hkv, scale):
    GW = rep * DH
    npairs = Hkv * B
    nsteps = npairs // NB
    rem = npairs - nsteps * NB
    f32 = jnp.float32
    bf16 = jnp.bfloat16

    def kv_copies(t, slot, n=NB):
        return (pltpu.make_async_copy(k_hbm.at[pl.ds(t * NB, n)], k_buf.at[slot, pl.ds(0, n)],
                                      k_sem.at[slot]),
                pltpu.make_async_copy(v_hbm.at[pl.ds(t * NB, n)], v_buf.at[slot, pl.ds(0, n)],
                                      v_sem.at[slot]))

    qoff = [sum(QW[:i]) for i in range(len(QW))]

    def wq_copy(ph):
        cols = pl.ds(qoff[ph] * GW, QW[ph] * GW)
        return pltpu.make_async_copy(wq_hbm.at[:, cols], wq_scr.at[:, cols], wq_sem.at[ph])

    x_copy = pltpu.make_async_copy(x_hbm, x_scr, x_sem)

    x_copy.start()
    wq_copy(0).start()

    st_scr[...] = jnp.ones(st_scr.shape, st_scr.dtype)

    x_copy.wait()
    for ph in range(len(QW)):
        wq_copy(ph).wait()
        if ph == 0:
            for p2 in range(1, len(QW)):
                wq_copy(p2).start()
            for c in kv_copies(0, 0):
                c.start()
        for g in range(qoff[ph], qoff[ph] + QW[ph]):
            q_all = jnp.dot(x_scr[...], wq_scr[:, g * GW:(g + 1) * GW], preferred_element_type=f32)
            q_all = (q_all * scale).astype(bf16)
            for bb in range(B):
                for r in range(rep):
                    qo_scr[bb * Hkv + g, r * Sq:(r + 1) * Sq, :] = (
                        q_all[bb * Sq:(bb + 1) * Sq, r * DH:(r + 1) * DH])
    for c in kv_copies(1, 1):
        c.start()

    def finalize(pair, i, z):
        l = jnp.sum(st_scr[2 * i + z], axis=-1, keepdims=True)
        r0 = pl.reciprocal(l, approx=True)
        inv = r0 * (2.0 - l * r0)
        qo_scr[pair] = (st_scr[2 * i + 1 + z] * inv).astype(bf16)

    def attend(pair0, slot, n, prev, z):
        fin = [[] for _ in range(n)]
        for ii in range(NB):
            fin[min(ii, n - 1)].append(ii)
        for i in range(n):
            sa = jax.lax.dot_general(qo_scr[pair0 + i], k_buf[slot, i, 0:QSPLIT, :], _NT,
                                     preferred_element_type=f32)
            for ii in fin[i]:
                finalize(prev + ii, ii, z)
            sb = jax.lax.dot_general(qo_scr[pair0 + i], k_buf[slot, i, QSPLIT:Sk, :], _NT,
                                     preferred_element_type=f32)
            s = jnp.concatenate([sa, sb], axis=1)
            m = jnp.max(s, axis=-1, keepdims=True)
            p = jnp.exp2(s - m)
            lp = p[:, 0:128]
            for tt in range(1, Sk // 128):
                lp = lp + p[:, tt * 128:(tt + 1) * 128]
            st_scr[2 * i] = lp
            st_scr[2 * i + 1] = jnp.dot(p.astype(bf16), v_buf[slot, i], preferred_element_type=f32)

    def step(t, carry):
        slot = jnp.bitwise_and(t, 1)
        z = jax.lax.shift_right_logical(t, 10)
        for c in kv_copies(t, slot):
            c.wait()
        prev = jnp.where(t > 0, (t - 1) * NB, npairs)
        attend(t * NB, slot, NB, prev, z)

        @pl.when(t + 2 < nsteps)
        def _():
            for c in kv_copies(t + 2, slot):
                c.start()

        if rem:
            @pl.when(t + 2 == nsteps)
            def _():
                for c in kv_copies(nsteps, nsteps % 2, rem):
                    c.start()

        @pl.when(t < NWO)
        def _():
            rows = pl.ds(pl.multiple_of(t * (HQ * DH // NWO), 16), HQ * DH // NWO)
            pltpu.make_async_copy(wo_hbm.at[rows], wo_scr.at[rows], wo_sem).start()
        return z

    z = jax.lax.fori_loop(0, nsteps, step, jnp.int32(0))

    pltpu.make_async_copy(wo_hbm, wo_scr, wo_sem).wait()
    if rem:
        for c in kv_copies(nsteps, nsteps % 2, rem):
            c.wait()
        attend(nsteps * NB, nsteps % 2, rem, (nsteps - 1) * NB + z, z)
        late = [(nsteps * NB + i, i) for i in range(rem)]
    else:
        late = [((nsteps - 1) * NB + i, i) for i in range(NB)]
    NW = D // OSPLIT

    def out_copy(n):
        cols = pl.ds(n * NW, NW)
        return pltpu.make_async_copy(out_scr.at[:, cols], out_hbm.at[:, cols], out_sem.at[n])

    for n in range(OSPLIT):
        acc = None
        for g in range(Hkv):
            if n == 0 and g == FING:
                for pair, i in late:
                    assert pair % Hkv >= FING
                    finalize(pair, i, z)
            o_g = jnp.concatenate(
                [jnp.concatenate([qo_scr[bb * Hkv + g, r * Sq:(r + 1) * Sq, :] for r in range(rep)],
                                 axis=1)
                 for bb in range(B)], axis=0)
            c = jnp.dot(o_g, wo_scr[g * GW:(g + 1) * GW, n * NW:(n + 1) * NW],
                        preferred_element_type=f32)
            acc = c if acc is None else acc + c
        out_scr[:, n * NW:(n + 1) * NW] = acc.astype(out_scr.dtype)
        out_copy(n).start()
    for n in range(OSPLIT):
        out_copy(n).wait()


@jax.jit
def pallas_standalone__gqa_block_cached__near_ridge_kernel(x, k_cache, v_cache, wq, wo):
    B, Sq, D = x.shape
    _, Hkv, Sk, Dh = k_cache.shape
    rep = HQ // Hkv
    M = rep * Sq
    assert Dh == DH and sum(QW) == Hkv and (B * Hkv) // NB >= NWO
    scale = (Dh ** -0.5) * math.log2(math.e)
    kern = functools.partial(_kernel, B=B, Sq=Sq, Sk=Sk, D=D, rep=rep, Hkv=Hkv, scale=scale)
    bf = jnp.bfloat16
    out = pl.pallas_call(
        kern,
        in_specs=[pl.BlockSpec(memory_space=pl.ANY)] * 5,
        out_specs=pl.BlockSpec(memory_space=pl.ANY),
        out_shape=jax.ShapeDtypeStruct((B * Sq, D), x.dtype),
        scratch_shapes=[
            pltpu.VMEM((B * Sq, D), bf),
            pltpu.VMEM((D, HQ * Dh), bf),
            pltpu.VMEM((HQ * Dh, D), bf),
            pltpu.VMEM((2, NB, Sk, Dh), bf),
            pltpu.VMEM((2, NB, Sk, Dh), bf),
            pltpu.VMEM((Hkv * B + NB, M, Dh), bf),
            pltpu.VMEM((2 * NB, M, Dh), jnp.float32),
            pltpu.VMEM((B * Sq, D), bf),
            pltpu.SemaphoreType.DMA(()),
            pltpu.SemaphoreType.DMA((len(QW),)),
            pltpu.SemaphoreType.DMA(()),
            pltpu.SemaphoreType.DMA((2,)),
            pltpu.SemaphoreType.DMA((2,)),
            pltpu.SemaphoreType.DMA((OSPLIT,)),
        ],
        compiler_params=pltpu.CompilerParams(
            vmem_limit_bytes=110 * 1024 * 1024,
            disable_bounds_checks=True,
        ),
    )(x.reshape(B * Sq, D), k_cache.reshape(B * Hkv, Sk, Dh), v_cache.reshape(B * Hkv, Sk, Dh), wq, wo)
    return out.reshape(B, Sq, D)
```

```python
import functools
import math

import jax
import jax.numpy as jnp
import jax.experimental.pallas as pl
import jax.experimental.pallas.tpu as pltpu

HQ = 32
DH = 128
R0 = 4
NB = 6
QH = (2, 3, 8, 19)
PING = 21
NWO = 8
CH = 512
FINC = 2
OSPLIT = 4
LSPLIT = 4
FING = 2

_NT = (((1,), (1,)), ((), ()))


def _kernel(x_hbm, k_hbm, v_hbm, wq_hbm, wo_hbm, out_hbm,
            x_scr, wq0, wq1, wq2, wq3, wo_scr, k_buf, v_buf, qo_scr, st_scr, out_scr,
            s_scr, m_scr0, m_scr1,
            x_sem, wq_sem, wo_sem, k_sem, v_sem, out_sem,
            *, B, Sq, Sk, D, rep, Hkv, scale):
    GW = rep * DH
    npairs = Hkv * B
    nsteps = (npairs - R0) // NB
    f32 = jnp.float32
    bf16 = jnp.bfloat16
    m_scr = (m_scr0, m_scr1)
    wq_scr = (wq0, wq1, wq2, wq3)
    hoff = [sum(QH[:i]) for i in range(len(QH) + 1)]
    HB = B // 2

    def kv_copies(pair0, slot, n=NB):
        return (pltpu.make_async_copy(k_hbm.at[pl.ds(pair0, n)], k_buf.at[slot, pl.ds(0, n)],
                                      k_sem.at[slot]),
                pltpu.make_async_copy(v_hbm.at[pl.ds(pair0, n)], v_buf.at[slot, pl.ds(0, n)],
                                      v_sem.at[slot]))

    def kv_start(pair0, slot, n=NB):
        for c in kv_copies(pair0, slot, n):
            c.start(priority=1)

    def kv_wait(pair0, slot, n=NB):
        for c in kv_copies(pair0, slot, n):
            c.wait()

    def wq_copy(ph):
        return pltpu.make_async_copy(wq_hbm.at[:, pl.ds(hoff[ph] * DH, QH[ph] * DH)],
                                     wq_scr[ph].at[:, pl.ds(0, QH[ph] * DH)], wq_sem.at[ph])

    def x_copy(h):
        rows = pl.ds(h * HB * Sq, HB * Sq)
        return pltpu.make_async_copy(x_hbm.at[rows], x_scr.at[rows], x_sem.at[h])

    def qproj(b0, b1, ph):
        h0, h1 = hoff[ph], hoff[ph + 1]
        for hh in range(h0, h1, rep):
            he = min(hh + rep, h1)
            q_all = jnp.dot(x_scr[b0 * Sq:b1 * Sq, :], wq_scr[ph][:, (hh - h0) * DH:(he - h0) * DH],
                            preferred_element_type=f32)
            q_all = (q_all * scale).astype(bf16)
            for bb in range(b0, b1):
                for h in range(hh, he):
                    qo_scr[bb * Hkv + h // rep, (h % rep) * Sq:(h % rep + 1) * Sq, :] = (
                        q_all[(bb - b0) * Sq:(bb - b0 + 1) * Sq, (h - hh) * DH:(h - hh + 1) * DH])
            if hh <= PING < he:
                k_buf[0, 0, 0:16, :] = q_all[0:16, 0:DH]
                v_buf[0, 0, 0:16, :] = q_all[0:16, 0:DH]
                kv_start(R0, 0)

    x_copy(0).start()
    wq_copy(0).start()
    x_copy(1).start(priority=1)
    st_scr[2 * R0:2 * NB] = jnp.ones((2 * (NB - R0),) + st_scr.shape[1:], f32)
    x_copy(0).wait()
    wq_copy(0).wait()
    wq_copy(1).start()
    wq_copy(2).start(priority=1)
    qproj(0, HB, 0)
    x_copy(1).wait()
    qproj(HB, B, 0)
    wq_copy(1).wait()
    wq_copy(3).start(priority=1)
    qproj(0, B, 1)
    wq_copy(2).wait()
    qproj(0, B, 2)
    wq_copy(3).wait()
    kv_start(0, 1, R0)
    qproj(0, B, 3)

    def finalize(pair, i, z):
        l = jnp.sum(st_scr[2 * i + z], axis=-1, keepdims=True)
        r0 = pl.reciprocal(l, approx=True)
        inv = r0 * (2.0 - l * r0)
        qo_scr[pair] = (st_scr[2 * i + 1 + z] * inv).astype(bf16)

    def attend(pair0, slot, n, prev, z):
        nc = Sk // CH
        for i in range(n):
            for c in range(nc):
                if c == FINC and prev is not None:
                    finalize(prev + i, i, z)
                s = jax.lax.dot_general(qo_scr[pair0 + i], k_buf[slot, i, c * CH:(c + 1) * CH, :],
                                        _NT, preferred_element_type=f32)
                if c < nc - 1:
                    s_scr[c] = s
                mp = None if c == 0 else m_scr[(c - 1) % 2][z]
                for tt in range(CH // 128):
                    st = s[:, tt * 128:(tt + 1) * 128]
                    mp = st if mp is None else jnp.maximum(mp, st)
                if c < nc - 1:
                    m_scr[c % 2][0] = mp
            m = jnp.max(mp, axis=-1, keepdims=True)
            s = jnp.concatenate([s_scr[c + z] for c in range(nc - 1)] + [s], axis=1)
            p = jnp.exp2(s - m)
            lp = p[:, 0:128]
            for tt in range(1, Sk // 128):
                lp = lp + p[:, tt * 128:(tt + 1) * 128]
            st_scr[2 * i] = lp
            st_scr[2 * i + 1] = jnp.dot(p.astype(bf16), v_buf[slot, i], preferred_element_type=f32)

    kv_wait(0, 1, R0)
    attend(0, 1, R0, None, 0)
    kv_start(R0 + NB, 1)

    def step(t, carry):
        slot = jnp.bitwise_and(t, 1)
        pair0 = R0 + t * NB
        kv_wait(pair0, slot)
        attend(pair0, slot, NB, jnp.maximum(pair0 - NB, 0), jax.lax.shift_right_logical(t, 10))

        @pl.when(t + 2 < nsteps)
        def _():
            kv_start(pair0 + 2 * NB, slot)

        @pl.when(t < NWO)
        def _():
            rows = pl.ds(pl.multiple_of(t * (HQ * DH // NWO), 16), HQ * DH // NWO)
            pltpu.make_async_copy(wo_hbm.at[rows], wo_scr.at[rows], wo_sem).start(priority=1)
        return carry

    jax.lax.fori_loop(0, nsteps, step, 0)

    pltpu.make_async_copy(wo_hbm, wo_scr, wo_sem).wait()
    NW = D // OSPLIT
    RQ = B * Sq // LSPLIT

    def out_copy(n, rq=None):
        cols = pl.ds(n * NW, NW)
        if rq is None:
            return pltpu.make_async_copy(out_scr.at[:, cols], out_hbm.at[:, cols], out_sem.at[n])
        rows = pl.ds(rq * RQ, RQ)
        return pltpu.make_async_copy(out_scr.at[rows, cols], out_hbm.at[rows, cols],
                                     out_sem.at[n + rq])

    for n in range(OSPLIT):
        acc = None
        for g in range(Hkv):
            if n == 0 and g == FING:
                for i in range(NB):
                    finalize(npairs - NB + i, i, 0)
            o_g = jnp.concatenate(
                [jnp.concatenate([qo_scr[bb * Hkv + g, r * Sq:(r + 1) * Sq, :] for r in range(rep)],
                                 axis=1)
                 for bb in range(B)], axis=0)
            c = jnp.dot(o_g, wo_scr[g * GW:(g + 1) * GW, n * NW:(n + 1) * NW],
                        preferred_element_type=f32)
            acc = c if acc is None else acc + c
        if n < OSPLIT - 1:
            out_scr[:, n * NW:(n + 1) * NW] = acc.astype(bf16)
            out_copy(n).start()
        else:
            for rq in range(LSPLIT):
                out_scr[rq * RQ:(rq + 1) * RQ, n * NW:(n + 1) * NW] = (
                    acc[rq * RQ:(rq + 1) * RQ].astype(bf16))
                out_copy(n, rq).start()
    for n in range(OSPLIT - 1):
        out_copy(n).wait()
    for rq in range(LSPLIT):
        out_copy(OSPLIT - 1, rq).wait()


@jax.jit
def pallas_standalone__gqa_block_cached__near_ridge_kernel(x, k_cache, v_cache, wq, wo):
    B, Sq, D = x.shape
    _, Hkv, Sk, Dh = k_cache.shape
    rep = HQ // Hkv
    M = rep * Sq
    npairs = B * Hkv
    assert Dh == DH and sum(QH) == HQ and B % 2 == 0 and Sk % CH == 0
    assert (npairs - R0) % NB == 0 and (npairs - R0) // NB >= max(NWO, 2)
    assert 0 < NB - R0 <= R0
    assert (npairs - NB) % Hkv >= FING and NB <= Hkv - FING
    assert QH[0] <= PING
    scale = (Dh ** -0.5) * math.log2(math.e)
    kern = functools.partial(_kernel, B=B, Sq=Sq, Sk=Sk, D=D, rep=rep, Hkv=Hkv, scale=scale)
    bf = jnp.bfloat16
    f32 = jnp.float32
    out = pl.pallas_call(
        kern,
        in_specs=[pl.BlockSpec(memory_space=pl.ANY)] * 5,
        out_specs=pl.BlockSpec(memory_space=pl.ANY),
        out_shape=jax.ShapeDtypeStruct((B * Sq, D), x.dtype),
        scratch_shapes=[
            pltpu.VMEM((B * Sq, D), bf),
            *[pltpu.VMEM((D, (n + 1) * Dh), bf) for n in QH],
            pltpu.VMEM((HQ * Dh, D), bf),
            pltpu.VMEM((2, NB, Sk, Dh), bf),
            pltpu.VMEM((2, NB, Sk, Dh), bf),
            pltpu.VMEM((npairs, M, Dh), bf),
            pltpu.VMEM((2 * NB, M, Dh), f32),
            pltpu.VMEM((B * Sq, D), bf),
            pltpu.VMEM((Sk // CH - 1, M, CH), f32),
            pltpu.VMEM((1, M, 128), f32),
            pltpu.VMEM((1, M, 128), f32),
            pltpu.SemaphoreType.DMA((2,)),
            pltpu.SemaphoreType.DMA((len(QH),)),
            pltpu.SemaphoreType.DMA(()),
            pltpu.SemaphoreType.DMA((2,)),
            pltpu.SemaphoreType.DMA((2,)),
            pltpu.SemaphoreType.DMA((OSPLIT - 1 + LSPLIT,)),
        ],
        compiler_params=pltpu.CompilerParams(
            vmem_limit_bytes=110 * 1024 * 1024,
            disable_bounds_checks=True,
            disable_semaphore_checks=True,
        ),
    )(x.reshape(B * Sq, D), k_cache.reshape(npairs, Sk, Dh), v_cache.reshape(npairs, Sk, Dh), wq, wo)
    return out.reshape(B, Sq, D)
```

```python
import functools
import math

import jax
import jax.numpy as jnp
import jax.experimental.pallas as pl
import jax.experimental.pallas.tpu as pltpu

HQ = 32
DH = 128
R0 = 4
NB = 6
QH = (2, 3, 8, 19)
PING = 21
NWO = 8
CH = 512
FINC = 2
TROW = 120
OSPLIT = 4
LSPLIT = 4
FING = 2

_NT = (((1,), (1,)), ((), ()))


def _kernel(x_hbm, k_hbm, v_hbm, wq_hbm, wo_hbm, out_hbm,
            x_scr, wq0, wq1, wq2, wq3, wo_scr, k_buf, v_buf, qo_scr, st_scr, out_scr,
            s_scr, sl_scr, m_scr0, m_scr1,
            x_sem, wq_sem, wo_sem, k_sem, v_sem, out_sem,
            *, B, Sq, Sk, D, rep, Hkv, scale):
    GW = rep * DH
    npairs = Hkv * B
    nsteps = (npairs - R0) // NB
    nc = Sk // CH
    f32 = jnp.float32
    bf16 = jnp.bfloat16
    m_scr = (m_scr0, m_scr1)
    wq_scr = (wq0, wq1, wq2, wq3)
    hoff = [sum(QH[:i]) for i in range(len(QH) + 1)]
    HB = B // 2

    def kv_copies(pair0, slot, n=NB):
        return (pltpu.make_async_copy(k_hbm.at[pl.ds(pair0, n)], k_buf.at[slot, pl.ds(0, n)],
                                      k_sem.at[slot]),
                pltpu.make_async_copy(v_hbm.at[pl.ds(pair0, n)], v_buf.at[slot, pl.ds(0, n)],
                                      v_sem.at[slot]))

    def kv_start(pair0, slot, n=NB):
        for c in kv_copies(pair0, slot, n):
            c.start(priority=1)

    def kv_wait(pair0, slot, n=NB):
        for c in kv_copies(pair0, slot, n):
            c.wait()

    def wq_copy(ph):
        return pltpu.make_async_copy(wq_hbm.at[:, pl.ds(hoff[ph] * DH, QH[ph] * DH)],
                                     wq_scr[ph].at[:, pl.ds(0, QH[ph] * DH)], wq_sem.at[ph])

    def x_copy(h):
        rows = pl.ds(h * HB * Sq, HB * Sq)
        return pltpu.make_async_copy(x_hbm.at[rows], x_scr.at[rows], x_sem.at[h])

    def qproj(b0, b1, ph):
        h0, h1 = hoff[ph], hoff[ph + 1]
        for hh in range(h0, h1, rep):
            he = min(hh + rep, h1)
            q_all = jnp.dot(x_scr[b0 * Sq:b1 * Sq, :], wq_scr[ph][:, (hh - h0) * DH:(he - h0) * DH],
                            preferred_element_type=f32)
            q_all = (q_all * scale).astype(bf16)
            for bb in range(b0, b1):
                for h in range(hh, he):
                    qo_scr[bb * Hkv + h // rep, (h % rep) * Sq:(h % rep + 1) * Sq, :] = (
                        q_all[(bb - b0) * Sq:(bb - b0 + 1) * Sq, (h - hh) * DH:(h - hh + 1) * DH])
            if hh <= PING < he:
                k_buf[0, 0, 0:16, :] = q_all[0:16, 0:DH]
                v_buf[0, 0, 0:16, :] = q_all[0:16, 0:DH]
                kv_start(R0, 0)

    x_copy(0).start()
    wq_copy(0).start()
    x_copy(1).start(priority=1)
    st_scr[2 * R0:2 * NB] = jnp.ones((2 * (NB - R0),) + st_scr.shape[1:], f32)
    z0 = jax.lax.fori_loop(0, 2, lambda i, c: jax.lax.shift_right_logical(i, 10), jnp.int32(0))
    x_copy(0).wait()
    wq_copy(0).wait()
    wq_copy(1).start()
    wq_copy(2).start(priority=1)
    qproj(0, HB, 0)
    x_copy(1).wait()
    qproj(HB, B, 0)
    wq_copy(1).wait()
    wq_copy(3).start(priority=1)
    qproj(0, B, 1)
    wq_copy(2).wait()
    qproj(0, B, 2)
    wq_copy(3).wait()
    kv_start(0, 1, R0)
    qproj(0, B, 3)

    def finalize(pair, i, z):
        l = jnp.sum(st_scr[2 * i + z], axis=-1, keepdims=True)
        r0 = pl.reciprocal(l, approx=True)
        inv = r0 * (2.0 - l * r0)
        qo_scr[pair] = (st_scr[2 * i + 1 + z] * inv).astype(bf16)

    def attend(pair0, slot, n, prev, z):
        for i in range(n):
            for c in range(nc):
                if c == FINC and prev is not None:
                    finalize(prev + i, i, z)
                s = jax.lax.dot_general(qo_scr[pair0 + i], k_buf[slot, i, c * CH:(c + 1) * CH, :],
                                        _NT, preferred_element_type=f32)
                mp = None if c == 0 else m_scr[(c - 1) % 2][z]
                for tt in range(CH // 128):
                    st = s[:, tt * 128:(tt + 1) * 128]
                    mp = st if mp is None else jnp.maximum(mp, st)
                if c < nc - 1:
                    s_scr[c] = s
                    m_scr[c % 2][0] = mp
                else:
                    sl_scr[0] = s
            m = jnp.max(mp, axis=-1, keepdims=True)
            lp = None
            acc = None
            for c in range(nc):
                p = jnp.exp2((s_scr[c + z] if c < nc - 1 else sl_scr[z]) - m)
                for tt in range(CH // 128):
                    pt = p[:, tt * 128:(tt + 1) * 128]
                    lp = pt if lp is None else lp + pt
                oc = jnp.dot(p.astype(bf16), v_buf[slot, i, c * CH:(c + 1) * CH, :],
                             preferred_element_type=f32)
                acc = oc if acc is None else acc + oc
                if c + 1 < nc - 1:
                    s_scr[nc - 1, 0:8, 0:128] = oc[TROW - 8:TROW]
                elif c + 1 < nc:
                    sl_scr[1, 0:8, 0:128] = oc[TROW - 8:TROW]
            st_scr[2 * i] = lp
            st_scr[2 * i + 1] = acc

    kv_wait(0, 1, R0)
    attend(0, 1, R0, None, z0)
    kv_start(R0 + NB, 1)

    def step(t, carry):
        slot = jnp.bitwise_and(t, 1)
        pair0 = R0 + t * NB
        kv_wait(pair0, slot)
        attend(pair0, slot, NB, jnp.maximum(pair0 - NB, 0), jax.lax.shift_right_logical(t, 10))

        @pl.when(t + 2 < nsteps)
        def _():
            kv_start(pair0 + 2 * NB, slot)

        @pl.when(t < NWO)
        def _():
            rows = pl.ds(pl.multiple_of(t * (HQ * DH // NWO), 16), HQ * DH // NWO)
            pltpu.make_async_copy(wo_hbm.at[rows], wo_scr.at[rows], wo_sem).start(priority=1)
        return carry

    jax.lax.fori_loop(0, nsteps, step, 0)

    pltpu.make_async_copy(wo_hbm, wo_scr, wo_sem).wait()
    NW = D // OSPLIT
    RQ = B * Sq // LSPLIT

    def out_copy(n, rq=None):
        cols = pl.ds(n * NW, NW)
        if rq is None:
            return pltpu.make_async_copy(out_scr.at[:, cols], out_hbm.at[:, cols], out_sem.at[n])
        rows = pl.ds(rq * RQ, RQ)
        return pltpu.make_async_copy(out_scr.at[rows, cols], out_hbm.at[rows, cols],
                                     out_sem.at[n + rq])

    for n in range(OSPLIT):
        acc = None
        for g in range(Hkv):
            if n == 0 and g == FING:
                for i in range(NB):
                    finalize(npairs - NB + i, i, 0)
            o_g = jnp.concatenate(
                [jnp.concatenate([qo_scr[bb * Hkv + g, r * Sq:(r + 1) * Sq, :] for r in range(rep)],
                                 axis=1)
                 for bb in range(B)], axis=0)
            c = jnp.dot(o_g, wo_scr[g * GW:(g + 1) * GW, n * NW:(n + 1) * NW],
                        preferred_element_type=f32)
            acc = c if acc is None else acc + c
        if n < OSPLIT - 1:
            out_scr[:, n * NW:(n + 1) * NW] = acc.astype(bf16)
            out_copy(n).start()
        else:
            for rq in range(LSPLIT):
                out_scr[rq * RQ:(rq + 1) * RQ, n * NW:(n + 1) * NW] = (
                    acc[rq * RQ:(rq + 1) * RQ].astype(bf16))
                out_copy(n, rq).start()
    for n in range(OSPLIT - 1):
        out_copy(n).wait()
    for rq in range(LSPLIT):
        out_copy(OSPLIT - 1, rq).wait()


@jax.jit
def pallas_standalone__gqa_block_cached__near_ridge_kernel(x, k_cache, v_cache, wq, wo):
    B, Sq, D = x.shape
    _, Hkv, Sk, Dh = k_cache.shape
    rep = HQ // Hkv
    M = rep * Sq
    npairs = B * Hkv
    assert Dh == DH and sum(QH) == HQ and B % 2 == 0 and Sk % CH == 0 and Sk // CH > FINC
    assert (npairs - R0) % NB == 0 and (npairs - R0) // NB >= max(NWO, 2)
    assert 0 < NB - R0 <= R0
    assert (npairs - NB) % Hkv >= FING and NB <= Hkv - FING
    assert QH[0] <= PING and 8 <= TROW <= M
    scale = (Dh ** -0.5) * math.log2(math.e)
    kern = functools.partial(_kernel, B=B, Sq=Sq, Sk=Sk, D=D, rep=rep, Hkv=Hkv, scale=scale)
    bf = jnp.bfloat16
    f32 = jnp.float32
    out = pl.pallas_call(
        kern,
        in_specs=[pl.BlockSpec(memory_space=pl.ANY)] * 5,
        out_specs=pl.BlockSpec(memory_space=pl.ANY),
        out_shape=jax.ShapeDtypeStruct((B * Sq, D), x.dtype),
        scratch_shapes=[
            pltpu.VMEM((B * Sq, D), bf),
            *[pltpu.VMEM((D, (n + 1) * Dh), bf) for n in QH],
            pltpu.VMEM((HQ * Dh, D), bf),
            pltpu.VMEM((2, NB, Sk, Dh), bf),
            pltpu.VMEM((2, NB, Sk, Dh), bf),
            pltpu.VMEM((npairs, M, Dh), bf),
            pltpu.VMEM((2 * NB, M, Dh), f32),
            pltpu.VMEM((B * Sq, D), bf),
            pltpu.VMEM((Sk // CH, M, CH), f32),
            pltpu.VMEM((2, M, CH), f32),
            pltpu.VMEM((1, M, 128), f32),
            pltpu.VMEM((1, M, 128), f32),
            pltpu.SemaphoreType.DMA((2,)),
            pltpu.SemaphoreType.DMA((len(QH),)),
            pltpu.SemaphoreType.DMA(()),
            pltpu.SemaphoreType.DMA((2,)),
            pltpu.SemaphoreType.DMA((2,)),
            pltpu.SemaphoreType.DMA((OSPLIT - 1 + LSPLIT,)),
        ],
        compiler_params=pltpu.CompilerParams(
            vmem_limit_bytes=110 * 1024 * 1024,
            disable_bounds_checks=True,
            disable_semaphore_checks=True,
        ),
    )(x.reshape(B * Sq, D), k_cache.reshape(npairs, Sk, Dh), v_cache.reshape(npairs, Sk, Dh), wq, wo)
    return out.reshape(B, Sq, D)
```

```python
import functools
import math

import jax
import jax.numpy as jnp
import jax.experimental.pallas as pl
import jax.experimental.pallas.tpu as pltpu

HQ = 32
DH = 128
R0 = 4
NB = 6
QH = (2, 3, 8, 19)
PING = 21
NWO = 8
CH = 512
FINC = 2
TROW = 120
OSPLIT = 4
LSPLIT = 4
FING = 2

_NT = (((1,), (1,)), ((), ()))


def _kernel(x_hbm, k_hbm, v_hbm, wq_hbm, wo_hbm, out_hbm,
            x_scr, wq0, wq1, wq2, wq3, wo_scr, k_buf, v_buf, qo_scr, st_scr, out_scr,
            s_scr, sl_scr, m_scr0, m_scr1, pt_scr, vt_scr,
            x_sem, wq_sem, wo_sem, k_sem, v_sem, out_sem,
            *, B, Sq, Sk, D, rep, Hkv, scale):
    GW = rep * DH
    npairs = Hkv * B
    nsteps = (npairs - R0) // NB
    nc = Sk // CH
    f32 = jnp.float32
    bf16 = jnp.bfloat16
    m_scr = (m_scr0, m_scr1)
    wq_scr = (wq0, wq1, wq2, wq3)
    hoff = [sum(QH[:i]) for i in range(len(QH) + 1)]
    HB = B // 2

    def kv_copies(pair0, slot, n=NB):
        return (pltpu.make_async_copy(k_hbm.at[pl.ds(pair0, n)], k_buf.at[slot, pl.ds(0, n)],
                                      k_sem.at[slot]),
                pltpu.make_async_copy(v_hbm.at[pl.ds(pair0, n)], v_buf.at[slot, pl.ds(0, n)],
                                      v_sem.at[slot]))

    def kv_start(pair0, slot, n=NB):
        for c in kv_copies(pair0, slot, n):
            c.start(priority=1)

    def kv_wait(pair0, slot, n=NB):
        for c in kv_copies(pair0, slot, n):
            c.wait()

    def wq_copy(ph):
        return pltpu.make_async_copy(wq_hbm.at[:, pl.ds(hoff[ph] * DH, QH[ph] * DH)],
                                     wq_scr[ph].at[:, pl.ds(0, QH[ph] * DH)], wq_sem.at[ph])

    def x_copy(h):
        rows = pl.ds(h * HB * Sq, HB * Sq)
        return pltpu.make_async_copy(x_hbm.at[rows], x_scr.at[rows], x_sem.at[h])

    def qproj(b0, b1, ph, first=0, last=None):
        h0, h1 = hoff[ph], hoff[ph + 1]
        for hh in list(range(h0, h1, rep))[first:last]:
            he = min(hh + rep, h1)
            q_all = jnp.dot(x_scr[b0 * Sq:b1 * Sq, :], wq_scr[ph][:, (hh - h0) * DH:(he - h0) * DH],
                            preferred_element_type=f32)
            q_all = (q_all * scale).astype(bf16)
            for bb in range(b0, b1):
                for h in range(hh, he):
                    qo_scr[bb * Hkv + h // rep, (h % rep) * Sq:(h % rep + 1) * Sq, :] = (
                        q_all[(bb - b0) * Sq:(bb - b0 + 1) * Sq, (h - hh) * DH:(h - hh + 1) * DH])
            if hh <= PING < he:
                k_buf[0, 0, 0:16, :] = q_all[0:16, 0:DH]
                v_buf[0, 0, 0:16, :] = q_all[0:16, 0:DH]
                kv_start(R0, 0)

    x_copy(0).start()
    wq_copy(0).start()
    x_copy(1).start(priority=1)
    st_scr[2 * R0:2 * NB] = jnp.ones((2 * (NB - R0),) + st_scr.shape[1:], f32)
    z0 = jax.lax.fori_loop(0, 2, lambda i, c: jax.lax.shift_right_logical(i, 10), jnp.int32(0))
    x_copy(0).wait()
    wq_copy(0).wait()
    wq_copy(1).start()
    wq_copy(2).start(priority=1)
    qproj(0, HB, 0)
    x_copy(1).wait()
    qproj(HB, B, 0)
    wq_copy(1).wait()
    wq_copy(3).start(priority=1)
    qproj(0, B, 1)
    wq_copy(2).wait()
    qproj(0, B, 2)
    wq_copy(3).wait()
    kv_start(0, 1, R0)
    qproj(0, B, 3, 0, -1)

    def finalize(pair, i, z):
        l = jnp.sum(st_scr[2 * i + z], axis=-1, keepdims=True)
        r0 = pl.reciprocal(l, approx=True)
        inv = r0 * (2.0 - l * r0)
        qo_scr[pair] = (st_scr[2 * i + 1 + z] * inv).astype(bf16)

    def attend(pair0, slot, n, prev, z):
        for i in range(n):
            for c in range(nc):
                if c == FINC and prev is not None:
                    finalize(prev + i, i, z)
                s = jax.lax.dot_general(qo_scr[pair0 + i], k_buf[slot, i, c * CH:(c + 1) * CH, :],
                                        _NT, preferred_element_type=f32)
                mp = None if c == 0 else m_scr[(c - 1) % 2][z]
                for tt in range(CH // 128):
                    st = s[:, tt * 128:(tt + 1) * 128]
                    mp = st if mp is None else jnp.maximum(mp, st)
                if c < nc - 1:
                    s_scr[c] = s
                    m_scr[c % 2][0] = mp
                else:
                    sl_scr[0] = s
            m = jnp.max(mp, axis=-1, keepdims=True)
            lp = None
            acc = None
            last = i == n - 1

            def ex(c):
                nonlocal lp
                p = jnp.exp2((s_scr[c + z] if c < nc - 1 else sl_scr[z]) - m)
                for tt in range(CH // 128):
                    pt = p[:, tt * 128:(tt + 1) * 128]
                    lp = pt if lp is None else lp + pt
                return p.astype(bf16)

            for c in range(nc - 1 if last else nc):
                oc = jnp.dot(ex(c), v_buf[slot, i, c * CH:(c + 1) * CH, :],
                             preferred_element_type=f32)
                acc = oc if acc is None else acc + oc
                if c + 1 < nc - 1:
                    s_scr[nc - 1, 0:8, 0:128] = oc[TROW - 8:TROW]
                elif c + 1 < nc and not last:
                    sl_scr[1, 0:8, 0:128] = oc[TROW - 8:TROW]
                if last and c == 0:
                    sl_scr[1, 0:8, 0:128] = oc[0:8]
                    pt_scr[0] = ex(nc - 1)
                    vt_scr[0] = v_buf[slot, i, (nc - 1) * CH:nc * CH, :]
            st_scr[2 * i] = lp
            st_scr[2 * i + 1] = acc

    def pv_tail(i, z):
        st_scr[2 * i + 1] = st_scr[2 * i + 1] + jnp.dot(pt_scr[z], vt_scr[z],
                                                        preferred_element_type=f32)

    kv_wait(0, 1, R0)
    qproj(0, B, 3, -1)
    attend(0, 1, R0, None, z0)
    kv_start(R0 + NB, 1)

    def step(t, carry):
        slot = jnp.bitwise_and(t, 1)
        pair0 = R0 + t * NB
        kv_wait(pair0, slot)
        z = jax.lax.shift_right_logical(t, 10)
        pv_tail(jnp.where(t > 0, NB - 1, R0 - 1), z)
        attend(pair0, slot, NB, jnp.maximum(pair0 - NB, 0), z)

        @pl.when(t + 2 < nsteps)
        def _():
            kv_start(pair0 + 2 * NB, slot)

        @pl.when(t < NWO)
        def _():
            rows = pl.ds(pl.multiple_of(t * (HQ * DH // NWO), 16), HQ * DH // NWO)
            pltpu.make_async_copy(wo_hbm.at[rows], wo_scr.at[rows], wo_sem).start(priority=1)
        return carry

    jax.lax.fori_loop(0, nsteps, step, 0)

    pltpu.make_async_copy(wo_hbm, wo_scr, wo_sem).wait()
    pv_tail(NB - 1, z0)
    NW = D // OSPLIT
    RQ = B * Sq // LSPLIT

    def out_copy(n, rq=None):
        cols = pl.ds(n * NW, NW)
        if rq is None:
            return pltpu.make_async_copy(out_scr.at[:, cols], out_hbm.at[:, cols], out_sem.at[n])
        rows = pl.ds(rq * RQ, RQ)
        return pltpu.make_async_copy(out_scr.at[rows, cols], out_hbm.at[rows, cols],
                                     out_sem.at[n + rq])

    for n in range(OSPLIT):
        acc = None
        for g in range(Hkv):
            if n == 0 and g == FING:
                for i in range(NB):
                    finalize(npairs - NB + i, i, 0)
            o_g = jnp.concatenate(
                [jnp.concatenate([qo_scr[bb * Hkv + g, r * Sq:(r + 1) * Sq, :] for r in range(rep)],
                                 axis=1)
                 for bb in range(B)], axis=0)
            c = jnp.dot(o_g, wo_scr[g * GW:(g + 1) * GW, n * NW:(n + 1) * NW],
                        preferred_element_type=f32)
            acc = c if acc is None else acc + c
        if n < OSPLIT - 1:
            out_scr[:, n * NW:(n + 1) * NW] = acc.astype(bf16)
            out_copy(n).start()
        else:
            for rq in range(LSPLIT):
                out_scr[rq * RQ:(rq + 1) * RQ, n * NW:(n + 1) * NW] = (
                    acc[rq * RQ:(rq + 1) * RQ].astype(bf16))
                out_copy(n, rq).start()
    for n in range(OSPLIT - 1):
        out_copy(n).wait()
    for rq in range(LSPLIT):
        out_copy(OSPLIT - 1, rq).wait()


@jax.jit
def pallas_standalone__gqa_block_cached__near_ridge_kernel(x, k_cache, v_cache, wq, wo):
    B, Sq, D = x.shape
    _, Hkv, Sk, Dh = k_cache.shape
    rep = HQ // Hkv
    M = rep * Sq
    npairs = B * Hkv
    assert Dh == DH and sum(QH) == HQ and B % 2 == 0 and Sk % CH == 0 and Sk // CH > FINC
    assert (npairs - R0) % NB == 0 and (npairs - R0) // NB >= max(NWO, 2)
    assert 0 < NB - R0 <= R0
    assert (npairs - NB) % Hkv >= FING and NB <= Hkv - FING
    assert QH[0] <= PING and 8 <= TROW <= M and Sk // CH >= 3
    assert R0 * rep <= HQ - rep
    scale = (Dh ** -0.5) * math.log2(math.e)
    kern = functools.partial(_kernel, B=B, Sq=Sq, Sk=Sk, D=D, rep=rep, Hkv=Hkv, scale=scale)
    bf = jnp.bfloat16
    f32 = jnp.float32
    out = pl.pallas_call(
        kern,
        in_specs=[pl.BlockSpec(memory_space=pl.ANY)] * 5,
        out_specs=pl.BlockSpec(memory_space=pl.ANY),
        out_shape=jax.ShapeDtypeStruct((B * Sq, D), x.dtype),
        scratch_shapes=[
            pltpu.VMEM((B * Sq, D), bf),
            *[pltpu.VMEM((D, (n + 1) * Dh), bf) for n in QH],
            pltpu.VMEM((HQ * Dh, D), bf),
            pltpu.VMEM((2, NB, Sk, Dh), bf),
            pltpu.VMEM((2, NB, Sk, Dh), bf),
            pltpu.VMEM((npairs, M, Dh), bf),
            pltpu.VMEM((2 * NB, M, Dh), f32),
            pltpu.VMEM((B * Sq, D), bf),
            pltpu.VMEM((Sk // CH, M, CH), f32),
            pltpu.VMEM((2, M, CH), f32),
            pltpu.VMEM((1, M, 128), f32),
            pltpu.VMEM((1, M, 128), f32),
            pltpu.VMEM((1, M, CH), bf),
            pltpu.VMEM((1, CH, Dh), bf),
            pltpu.SemaphoreType.DMA((2,)),
            pltpu.SemaphoreType.DMA((len(QH),)),
            pltpu.SemaphoreType.DMA(()),
            pltpu.SemaphoreType.DMA((2,)),
            pltpu.SemaphoreType.DMA((2,)),
            pltpu.SemaphoreType.DMA((OSPLIT - 1 + LSPLIT,)),
        ],
        compiler_params=pltpu.CompilerParams(
            vmem_limit_bytes=110 * 1024 * 1024,
            disable_bounds_checks=True,
            disable_semaphore_checks=True,
        ),
    )(x.reshape(B * Sq, D), k_cache.reshape(npairs, Sk, Dh), v_cache.reshape(npairs, Sk, Dh), wq, wo)
    return out.reshape(B, Sq, D)
```

```python
import functools
import math

import jax
import jax.numpy as jnp
import jax.experimental.pallas as pl
import jax.experimental.pallas.tpu as pltpu

HQ = 32
DH = 128
R0 = 4
NB = 6
QH = (8, 11, 8, 5)
KS = (128, 128, 256)
PING = 21
NWO = 8
CH = 512
FINC = 2
TROW = 120
OSPLIT = 4
LSPLIT = 4
FING = 2

_NT = (((1,), (1,)), ((), ()))


def _kernel(x_hbm, k_hbm, v_hbm, wq_hbm, wo_hbm, out_hbm,
            x_scr, wq0, wq1, wq2, wq3, wo_scr, k_buf, v_buf, qo_scr, st_scr, out_scr,
            s_scr, sl_scr, m_scr0, m_scr1, pt_scr, vt_scr, qa_scr,
            x_sem, wk_sem, wq_sem, wo_sem, k_sem, v_sem, out_sem,
            *, B, Sq, Sk, D, rep, Hkv, scale):
    GW = rep * DH
    npairs = Hkv * B
    nsteps = (npairs - R0) // NB
    nc = Sk // CH
    f32 = jnp.float32
    bf16 = jnp.bfloat16
    m_scr = (m_scr0, m_scr1)
    wq_scr = (wq0, wq1, wq2, wq3)
    hoff = [sum(QH[:i]) for i in range(len(QH) + 1)]
    koff = [sum(KS[:i]) for i in range(len(KS) + 1)]

    def kv_copies(pair0, slot, n=NB):
        return (pltpu.make_async_copy(k_hbm.at[pl.ds(pair0, n)], k_buf.at[slot, pl.ds(0, n)],
                                      k_sem.at[slot]),
                pltpu.make_async_copy(v_hbm.at[pl.ds(pair0, n)], v_buf.at[slot, pl.ds(0, n)],
                                      v_sem.at[slot]))

    def kv_start(pair0, slot, n=NB):
        for c in kv_copies(pair0, slot, n):
            c.start(priority=1)

    def kv_wait(pair0, slot, n=NB):
        for c in kv_copies(pair0, slot, n):
            c.wait()

    def wq_copy(ph):
        return pltpu.make_async_copy(wq_hbm.at[:, pl.ds(hoff[ph] * DH, QH[ph] * DH)],
                                     wq_scr[ph].at[:, pl.ds(0, QH[ph] * DH)], wq_sem.at[ph])

    def k_copies(j):
        ks = pl.ds(koff[j], KS[j])
        cols = pl.ds(0, QH[0] * DH)
        return (pltpu.make_async_copy(x_hbm.at[:, ks], x_scr.at[:, ks], x_sem.at[j]),
                pltpu.make_async_copy(wq_hbm.at[ks, cols], wq_scr[0].at[ks, cols], wk_sem.at[j]))

    def q_store(q_all, hh, he):
        q_all = (q_all * scale).astype(bf16)
        for bb in range(B):
            for h in range(hh, he):
                qo_scr[bb * Hkv + h // rep, (h % rep) * Sq:(h % rep + 1) * Sq, :] = (
                    q_all[bb * Sq:(bb + 1) * Sq, (h - hh) * DH:(h - hh + 1) * DH])
        return q_all

    def qproj(ph):
        h0, h1 = hoff[ph], hoff[ph + 1]
        for hh in range(h0, h1, rep):
            he = min(hh + rep, h1)
            q_all = q_store(jnp.dot(x_scr[...], wq_scr[ph][:, (hh - h0) * DH:(he - h0) * DH],
                                    preferred_element_type=f32), hh, he)
            if hh <= PING < he:
                k_buf[0, 0, 0:16, :] = q_all[0:16, 0:DH]
                v_buf[0, 0, 0:16, :] = q_all[0:16, 0:DH]
                kv_start(R0, 0)

    for j in range(len(KS)):
        for c in k_copies(j):
            c.start()
    st_scr[2 * R0:2 * NB] = jnp.ones((2 * (NB - R0),) + st_scr.shape[1:], f32)
    z0 = jax.lax.fori_loop(0, 2, lambda i, c: jax.lax.shift_right_logical(i, 10), jnp.int32(0))
    for j in range(len(KS)):
        for c in k_copies(j):
            c.wait()
        if j == 0:
            wq_copy(1).start(priority=1)
        if j == len(KS) - 1:
            wq_copy(2).start(priority=1)
        part = jnp.dot(x_scr[:, koff[j]:koff[j + 1]], wq_scr[0][koff[j]:koff[j + 1], 0:QH[0] * DH],
                       preferred_element_type=f32)
        if j > 0:
            part = part + qa_scr[...]
        if j < len(KS) - 1:
            qa_scr[...] = part
        else:
            q_store(part, 0, QH[0])
    wq_copy(1).wait()
    wq_copy(3).start(priority=1)
    kv_start(0, 1, R0)
    qproj(1)
    wq_copy(2).wait()
    qproj(2)

    def finalize(pair, i, z):
        l = jnp.sum(st_scr[2 * i + z], axis=-1, keepdims=True)
        r0 = pl.reciprocal(l, approx=True)
        inv = r0 * (2.0 - l * r0)
        qo_scr[pair] = (st_scr[2 * i + 1 + z] * inv).astype(bf16)

    def attend(pair0, slot, n, prev, z):
        for i in range(n):
            for c in range(nc):
                if c == FINC and prev is not None:
                    finalize(prev + i, i, z)
                s = jax.lax.dot_general(qo_scr[pair0 + i], k_buf[slot, i, c * CH:(c + 1) * CH, :],
                                        _NT, preferred_element_type=f32)
                mp = None if c == 0 else m_scr[(c - 1) % 2][z]
                for tt in range(CH // 128):
                    st = s[:, tt * 128:(tt + 1) * 128]
                    mp = st if mp is None else jnp.maximum(mp, st)
                if c < nc - 1:
                    s_scr[c] = s
                    m_scr[c % 2][0] = mp
                else:
                    sl_scr[0] = s
            m = jnp.max(mp, axis=-1, keepdims=True)
            lp = None
            acc = None
            last = i == n - 1

            def ex(c):
                nonlocal lp
                p = jnp.exp2((s_scr[c + z] if c < nc - 1 else sl_scr[z]) - m)
                for tt in range(CH // 128):
                    pt = p[:, tt * 128:(tt + 1) * 128]
                    lp = pt if lp is None else lp + pt
                return p.astype(bf16)

            for c in range(nc - 1 if last else nc):
                oc = jnp.dot(ex(c), v_buf[slot, i, c * CH:(c + 1) * CH, :],
                             preferred_element_type=f32)
                acc = oc if acc is None else acc + oc
                if c + 1 < nc - 1:
                    s_scr[nc - 1, 0:8, 0:128] = oc[TROW - 8:TROW]
                elif c + 1 < nc and not last:
                    sl_scr[1, 0:8, 0:128] = oc[TROW - 8:TROW]
                if last and c == 0:
                    sl_scr[1, 0:8, 0:128] = oc[0:8]
                    pt_scr[0] = ex(nc - 1)
                    vt_scr[0] = v_buf[slot, i, (nc - 1) * CH:nc * CH, :]
            st_scr[2 * i] = lp
            st_scr[2 * i + 1] = acc

    def pv_tail(i, z):
        st_scr[2 * i + 1] = st_scr[2 * i + 1] + jnp.dot(pt_scr[z], vt_scr[z],
                                                        preferred_element_type=f32)

    wq_copy(3).wait()
    kv_wait(0, 1, R0)
    qproj(3)
    attend(0, 1, R0, None, z0)
    kv_start(R0 + NB, 1)

    def step(t, carry):
        slot = jnp.bitwise_and(t, 1)
        pair0 = R0 + t * NB
        kv_wait(pair0, slot)
        z = jax.lax.shift_right_logical(t, 10)
        pv_tail(jnp.where(t > 0, NB - 1, R0 - 1), z)
        attend(pair0, slot, NB, jnp.maximum(pair0 - NB, 0), z)

        @pl.when(t + 2 < nsteps)
        def _():
            kv_start(pair0 + 2 * NB, slot)

        @pl.when(t < NWO)
        def _():
            rows = pl.ds(pl.multiple_of(t * (HQ * DH // NWO), 16), HQ * DH // NWO)
            pltpu.make_async_copy(wo_hbm.at[rows], wo_scr.at[rows], wo_sem).start(priority=1)
        return carry

    jax.lax.fori_loop(0, nsteps, step, 0)

    pltpu.make_async_copy(wo_hbm, wo_scr, wo_sem).wait()
    pv_tail(NB - 1, z0)
    NW = D // OSPLIT
    RQ = B * Sq // LSPLIT

    def out_copy(n, rq=None):
        cols = pl.ds(n * NW, NW)
        if rq is None:
            return pltpu.make_async_copy(out_scr.at[:, cols], out_hbm.at[:, cols], out_sem.at[n])
        rows = pl.ds(rq * RQ, RQ)
        return pltpu.make_async_copy(out_scr.at[rows, cols], out_hbm.at[rows, cols],
                                     out_sem.at[n + rq])

    for n in range(OSPLIT):
        acc = None
        for g in range(Hkv):
            if n == 0 and g == FING:
                for i in range(NB):
                    finalize(npairs - NB + i, i, 0)
            o_g = jnp.concatenate(
                [jnp.concatenate([qo_scr[bb * Hkv + g, r * Sq:(r + 1) * Sq, :] for r in range(rep)],
                                 axis=1)
                 for bb in range(B)], axis=0)
            c = jnp.dot(o_g, wo_scr[g * GW:(g + 1) * GW, n * NW:(n + 1) * NW],
                        preferred_element_type=f32)
            acc = c if acc is None else acc + c
        if n < OSPLIT - 1:
            out_scr[:, n * NW:(n + 1) * NW] = acc.astype(bf16)
            out_copy(n).start()
        else:
            for rq in range(LSPLIT):
                out_scr[rq * RQ:(rq + 1) * RQ, n * NW:(n + 1) * NW] = (
                    acc[rq * RQ:(rq + 1) * RQ].astype(bf16))
                out_copy(n, rq).start()
    for n in range(OSPLIT - 1):
        out_copy(n).wait()
    for rq in range(LSPLIT):
        out_copy(OSPLIT - 1, rq).wait()


@jax.jit
def pallas_standalone__gqa_block_cached__near_ridge_kernel(x, k_cache, v_cache, wq, wo):
    B, Sq, D = x.shape
    _, Hkv, Sk, Dh = k_cache.shape
    rep = HQ // Hkv
    M = rep * Sq
    npairs = B * Hkv
    assert Dh == DH and sum(QH) == HQ and sum(KS) == D and Sk % CH == 0 and Sk // CH > FINC
    assert (npairs - R0) % NB == 0 and (npairs - R0) // NB >= max(NWO, 2)
    assert 0 < NB - R0 <= R0
    assert (npairs - NB) % Hkv >= FING and NB <= Hkv - FING
    assert QH[0] <= PING < HQ - QH[-1] and 8 <= TROW <= M and Sk // CH >= 3
    scale = (Dh ** -0.5) * math.log2(math.e)
    kern = functools.partial(_kernel, B=B, Sq=Sq, Sk=Sk, D=D, rep=rep, Hkv=Hkv, scale=scale)
    bf = jnp.bfloat16
    f32 = jnp.float32
    out = pl.pallas_call(
        kern,
        in_specs=[pl.BlockSpec(memory_space=pl.ANY)] * 5,
        out_specs=pl.BlockSpec(memory_space=pl.ANY),
        out_shape=jax.ShapeDtypeStruct((B * Sq, D), x.dtype),
        scratch_shapes=[
            pltpu.VMEM((B * Sq, D), bf),
            *[pltpu.VMEM((D, (n + 1) * Dh), bf) for n in QH],
            pltpu.VMEM((HQ * Dh, D), bf),
            pltpu.VMEM((2, NB, Sk, Dh), bf),
            pltpu.VMEM((2, NB, Sk, Dh), bf),
            pltpu.VMEM((npairs, M, Dh), bf),
            pltpu.VMEM((2 * NB, M, Dh), f32),
            pltpu.VMEM((B * Sq, D), bf),
            pltpu.VMEM((Sk // CH, M, CH), f32),
            pltpu.VMEM((2, M, CH), f32),
            pltpu.VMEM((1, M, 128), f32),
            pltpu.VMEM((1, M, 128), f32),
            pltpu.VMEM((1, M, CH), bf),
            pltpu.VMEM((1, CH, Dh), bf),
            pltpu.VMEM((B * Sq, QH[0] * Dh), f32),
            pltpu.SemaphoreType.DMA((len(KS),)),
            pltpu.SemaphoreType.DMA((len(KS),)),
            pltpu.SemaphoreType.DMA((len(QH),)),
            pltpu.SemaphoreType.DMA(()),
            pltpu.SemaphoreType.DMA((2,)),
            pltpu.SemaphoreType.DMA((2,)),
            pltpu.SemaphoreType.DMA((OSPLIT - 1 + LSPLIT,)),
        ],
        compiler_params=pltpu.CompilerParams(
            vmem_limit_bytes=110 * 1024 * 1024,
            disable_bounds_checks=True,
            disable_semaphore_checks=True,
        ),
    )(x.reshape(B * Sq, D), k_cache.reshape(npairs, Sk, Dh), v_cache.reshape(npairs, Sk, Dh), wq, wo)
    return out.reshape(B, Sq, D)
```

```python
import functools
import math

import jax
import jax.numpy as jnp
import jax.experimental.pallas as pl
import jax.experimental.pallas.tpu as pltpu

HQ = 32
DH = 128
R0 = 4
NB = 6
QH = (8, 10, 10, 4)
KS = (128, 128, 256)
NWO = 8
CH = 512
FINC = 2
TROW = 120
OSPLIT = 4
LSPLIT = 4
FING = 2

_NT = (((1,), (1,)), ((), ()))


def _kernel(x_hbm, k_hbm, v_hbm, wq_hbm, wo_hbm, out_hbm,
            x_scr, wq0, wq1, wq2, wq3, wo_scr, k_buf, v_buf, qo_scr, st_scr, out_scr,
            s_scr, sl_scr, m_scr0, m_scr1, pt_scr, vt_scr, qa_scr,
            x_sem, wk_sem, wq_sem, wo_sem, k_sem, v_sem, out_sem,
            *, B, Sq, Sk, D, rep, Hkv, scale):
    GW = rep * DH
    npairs = Hkv * B
    nsteps = (npairs - R0) // NB
    nc = Sk // CH
    f32 = jnp.float32
    bf16 = jnp.bfloat16
    m_scr = (m_scr0, m_scr1)
    wq_scr = (wq0, wq1, wq2, wq3)
    hoff = [sum(QH[:i]) for i in range(len(QH) + 1)]
    koff = [sum(KS[:i]) for i in range(len(KS) + 1)]

    def kv_copies(pair0, slot, n=NB):
        return (pltpu.make_async_copy(k_hbm.at[pl.ds(pair0, n)], k_buf.at[slot, pl.ds(0, n)],
                                      k_sem.at[slot]),
                pltpu.make_async_copy(v_hbm.at[pl.ds(pair0, n)], v_buf.at[slot, pl.ds(0, n)],
                                      v_sem.at[slot]))

    def kv_start(pair0, slot, n=NB):
        for c in kv_copies(pair0, slot, n):
            c.start(priority=1)

    def kv_wait(pair0, slot, n=NB):
        for c in kv_copies(pair0, slot, n):
            c.wait()

    def wq_copy(ph):
        return pltpu.make_async_copy(wq_hbm.at[:, pl.ds(hoff[ph] * DH, QH[ph] * DH)],
                                     wq_scr[ph].at[:, pl.ds(0, QH[ph] * DH)], wq_sem.at[ph])

    def k_copies(j):
        ks = pl.ds(koff[j], KS[j])
        cols = pl.ds(0, QH[0] * DH)
        return (pltpu.make_async_copy(x_hbm.at[:, ks], x_scr.at[:, ks], x_sem.at[j]),
                pltpu.make_async_copy(wq_hbm.at[ks, cols], wq_scr[0].at[ks, cols], wk_sem.at[j]))

    def q_store(q_all, hh, he):
        q_all = (q_all * scale).astype(bf16)
        for bb in range(B):
            for h in range(hh, he):
                qo_scr[bb * Hkv + h // rep, (h % rep) * Sq:(h % rep + 1) * Sq, :] = (
                    q_all[bb * Sq:(bb + 1) * Sq, (h - hh) * DH:(h - hh + 1) * DH])

    def qproj(ph):
        h0, h1 = hoff[ph], hoff[ph + 1]
        for hh in range(h0, h1, rep):
            he = min(hh + rep, h1)
            q_store(jnp.dot(x_scr[...], wq_scr[ph][:, (hh - h0) * DH:(he - h0) * DH],
                            preferred_element_type=f32), hh, he)

    for j in range(len(KS)):
        for c in k_copies(j):
            c.start()
    st_scr[2 * R0:2 * NB] = jnp.ones((2 * (NB - R0),) + st_scr.shape[1:], f32)
    z0 = jax.lax.fori_loop(0, 2, lambda i, c: jax.lax.shift_right_logical(i, 10), jnp.int32(0))
    for j in range(len(KS)):
        for c in k_copies(j):
            c.wait()
        if j == 0:
            wq_copy(1).start(priority=1)
        if j == len(KS) - 1:
            wq_copy(2).start(priority=1)
        part = jnp.dot(x_scr[:, koff[j]:koff[j + 1]], wq_scr[0][koff[j]:koff[j + 1], 0:QH[0] * DH],
                       preferred_element_type=f32)
        if j > 0:
            part = part + qa_scr[...]
        if j < len(KS) - 1:
            qa_scr[...] = part
        else:
            q_store(part, 0, QH[0])
    wq_copy(1).wait()
    wq_copy(3).start(priority=1)
    kv_start(0, 1, R0)
    qproj(1)
    wq_copy(2).wait()
    kv_start(R0, 0)
    qproj(2)

    def finalize(pair, i, z):
        l = jnp.sum(st_scr[2 * i + z], axis=-1, keepdims=True)
        r0 = pl.reciprocal(l, approx=True)
        inv = r0 * (2.0 - l * r0)
        qo_scr[pair] = (st_scr[2 * i + 1 + z] * inv).astype(bf16)

    def attend(pair0, slot, n, prev, z):
        for i in range(n):
            for c in range(nc):
                if c == FINC and prev is not None:
                    finalize(prev + i, i, z)
                s = jax.lax.dot_general(qo_scr[pair0 + i], k_buf[slot, i, c * CH:(c + 1) * CH, :],
                                        _NT, preferred_element_type=f32)
                mp = None if c == 0 else m_scr[(c - 1) % 2][z]
                for tt in range(CH // 128):
                    st = s[:, tt * 128:(tt + 1) * 128]
                    mp = st if mp is None else jnp.maximum(mp, st)
                if c < nc - 1:
                    s_scr[c] = s
                    m_scr[c % 2][0] = mp
                else:
                    sl_scr[0] = s
            m = jnp.max(mp, axis=-1, keepdims=True)
            lp = None
            acc = None
            last = i == n - 1

            def ex(c):
                nonlocal lp
                p = jnp.exp2((s_scr[c + z] if c < nc - 1 else sl_scr[z]) - m)
                for tt in range(CH // 128):
                    pt = p[:, tt * 128:(tt + 1) * 128]
                    lp = pt if lp is None else lp + pt
                return p.astype(bf16)

            for c in range(nc - 1 if last else nc):
                oc = jnp.dot(ex(c), v_buf[slot, i, c * CH:(c + 1) * CH, :],
                             preferred_element_type=f32)
                acc = oc if acc is None else acc + oc
                if c + 1 < nc - 1:
                    s_scr[nc - 1, 0:8, 0:128] = oc[TROW - 8:TROW]
                elif c + 1 < nc and not last:
                    sl_scr[1, 0:8, 0:128] = oc[TROW - 8:TROW]
                if last and c == 0:
                    sl_scr[1, 0:8, 0:128] = oc[0:8]
                    pt_scr[0] = ex(nc - 1)
                    vt_scr[0] = v_buf[slot, i, (nc - 1) * CH:nc * CH, :]
            st_scr[2 * i] = lp
            st_scr[2 * i + 1] = acc

    def pv_tail(i, z):
        st_scr[2 * i + 1] = st_scr[2 * i + 1] + jnp.dot(pt_scr[z], vt_scr[z],
                                                        preferred_element_type=f32)

    wq_copy(3).wait()
    kv_wait(0, 1, R0)
    qproj(3)
    attend(0, 1, R0, None, z0)
    kv_start(R0 + NB, 1)

    def step(t, carry):
        slot = jnp.bitwise_and(t, 1)
        pair0 = R0 + t * NB
        kv_wait(pair0, slot)
        z = jax.lax.shift_right_logical(t, 10)
        pv_tail(jnp.where(t > 0, NB - 1, R0 - 1), z)
        attend(pair0, slot, NB, jnp.maximum(pair0 - NB, 0), z)

        @pl.when(t + 2 < nsteps)
        def _():
            kv_start(pair0 + 2 * NB, slot)

        @pl.when(t < NWO)
        def _():
            rows = pl.ds(pl.multiple_of(t * (HQ * DH // NWO), 16), HQ * DH // NWO)
            pltpu.make_async_copy(wo_hbm.at[rows], wo_scr.at[rows], wo_sem).start(priority=1)
        return carry

    jax.lax.fori_loop(0, nsteps, step, 0)

    pltpu.make_async_copy(wo_hbm, wo_scr, wo_sem).wait()
    pv_tail(NB - 1, z0)
    NW = D // OSPLIT
    RQ = B * Sq // LSPLIT

    def out_copy(n, rq=None):
        cols = pl.ds(n * NW, NW)
        if rq is None:
            return pltpu.make_async_copy(out_scr.at[:, cols], out_hbm.at[:, cols], out_sem.at[n])
        rows = pl.ds(rq * RQ, RQ)
        return pltpu.make_async_copy(out_scr.at[rows, cols], out_hbm.at[rows, cols],
                                     out_sem.at[n + rq])

    for n in range(OSPLIT):
        acc = None
        for g in range(Hkv):
            if n == 0 and g == FING:
                for i in range(NB):
                    finalize(npairs - NB + i, i, 0)
            o_g = jnp.concatenate(
                [jnp.concatenate([qo_scr[bb * Hkv + g, r * Sq:(r + 1) * Sq, :] for r in range(rep)],
                                 axis=1)
                 for bb in range(B)], axis=0)
            c = jnp.dot(o_g, wo_scr[g * GW:(g + 1) * GW, n * NW:(n + 1) * NW],
                        preferred_element_type=f32)
            acc = c if acc is None else acc + c
        if n < OSPLIT - 1:
            out_scr[:, n * NW:(n + 1) * NW] = acc.astype(bf16)
            out_copy(n).start()
        else:
            for rq in range(LSPLIT):
                out_scr[rq * RQ:(rq + 1) * RQ, n * NW:(n + 1) * NW] = (
                    acc[rq * RQ:(rq + 1) * RQ].astype(bf16))
                out_copy(n, rq).start()
    for n in range(OSPLIT - 1):
        out_copy(n).wait()
    for rq in range(LSPLIT):
        out_copy(OSPLIT - 1, rq).wait()


@jax.jit
def pallas_standalone__gqa_block_cached__near_ridge_kernel(x, k_cache, v_cache, wq, wo):
    B, Sq, D = x.shape
    _, Hkv, Sk, Dh = k_cache.shape
    rep = HQ // Hkv
    M = rep * Sq
    npairs = B * Hkv
    assert Dh == DH and sum(QH) == HQ and sum(KS) == D and Sk % CH == 0 and Sk // CH > FINC
    assert (npairs - R0) % NB == 0 and (npairs - R0) // NB >= max(NWO, 2)
    assert 0 < NB - R0 <= R0
    assert (npairs - NB) % Hkv >= FING and NB <= Hkv - FING
    assert 8 <= TROW <= M and Sk // CH >= 3
    scale = (Dh ** -0.5) * math.log2(math.e)
    kern = functools.partial(_kernel, B=B, Sq=Sq, Sk=Sk, D=D, rep=rep, Hkv=Hkv, scale=scale)
    bf = jnp.bfloat16
    f32 = jnp.float32
    out = pl.pallas_call(
        kern,
        in_specs=[pl.BlockSpec(memory_space=pl.ANY)] * 5,
        out_specs=pl.BlockSpec(memory_space=pl.ANY),
        out_shape=jax.ShapeDtypeStruct((B * Sq, D), x.dtype),
        scratch_shapes=[
            pltpu.VMEM((B * Sq, D), bf),
            *[pltpu.VMEM((D, (n + 1) * Dh), bf) for n in QH],
            pltpu.VMEM((HQ * Dh, D), bf),
            pltpu.VMEM((2, NB, Sk, Dh), bf),
            pltpu.VMEM((2, NB, Sk, Dh), bf),
            pltpu.VMEM((npairs, M, Dh), bf),
            pltpu.VMEM((2 * NB, M, Dh), f32),
            pltpu.VMEM((B * Sq, D), bf),
            pltpu.VMEM((Sk // CH, M, CH), f32),
            pltpu.VMEM((2, M, CH), f32),
            pltpu.VMEM((1, M, 128), f32),
            pltpu.VMEM((1, M, 128), f32),
            pltpu.VMEM((1, M, CH), bf),
            pltpu.VMEM((1, CH, Dh), bf),
            pltpu.VMEM((B * Sq, QH[0] * Dh), f32),
            pltpu.SemaphoreType.DMA((len(KS),)),
            pltpu.SemaphoreType.DMA((len(KS),)),
            pltpu.SemaphoreType.DMA((len(QH),)),
            pltpu.SemaphoreType.DMA(()),
            pltpu.SemaphoreType.DMA((2,)),
            pltpu.SemaphoreType.DMA((2,)),
            pltpu.SemaphoreType.DMA((OSPLIT - 1 + LSPLIT,)),
        ],
        compiler_params=pltpu.CompilerParams(
            vmem_limit_bytes=110 * 1024 * 1024,
            disable_bounds_checks=True,
            disable_semaphore_checks=True,
        ),
    )(x.reshape(B * Sq, D), k_cache.reshape(npairs, Sk, Dh), v_cache.reshape(npairs, Sk, Dh), wq, wo)
    return out.reshape(B, Sq, D)
```

```python
import functools
import math

import jax
import jax.numpy as jnp
import jax.experimental.pallas as pl
import jax.experimental.pallas.tpu as pltpu

HQ = 32
DH = 128
R0 = 4
NB = 6
QH = (8, 10, 10, 4)
KS = (128, 128, 256)
NWO = 8
CH = 512
FINC = 2
TROW = 120
OSPLIT = 4
LSPLIT = 4
FING = 2

_NT = (((1,), (1,)), ((), ()))


def _kernel(x_hbm, k_hbm, v_hbm, wq_hbm, wo_hbm, out_hbm,
            x_scr, wq0, wq1, wq2, wq3, wo_scr, k_buf, v_buf, qo_scr, st_scr, out_scr,
            s_scr, sl_scr, m_scr0, m_scr1, pt_scr, vt_scr, qa_scr,
            x_sem, wk_sem, wq_sem, wo_sem, k_sem, v_sem, out_sem,
            *, B, Sq, Sk, D, rep, Hkv, scale):
    GW = rep * DH
    npairs = Hkv * B
    nsteps = (npairs - R0) // NB
    nc = Sk // CH
    f32 = jnp.float32
    bf16 = jnp.bfloat16
    m_scr = (m_scr0, m_scr1)
    wq_scr = (wq0, wq1, wq2, wq3)
    hoff = [sum(QH[:i]) for i in range(len(QH) + 1)]
    koff = [sum(KS[:i]) for i in range(len(KS) + 1)]

    def kv_copies(pair0, slot, n=NB):
        return (pltpu.make_async_copy(k_hbm.at[pl.ds(pair0, n)], k_buf.at[slot, pl.ds(0, n)],
                                      k_sem.at[slot]),
                pltpu.make_async_copy(v_hbm.at[pl.ds(pair0, n)], v_buf.at[slot, pl.ds(0, n)],
                                      v_sem.at[slot]))

    def kv_start(pair0, slot, n=NB):
        for c in kv_copies(pair0, slot, n):
            c.start(priority=1)

    def kv_wait(pair0, slot, n=NB):
        for c in kv_copies(pair0, slot, n):
            c.wait()

    def wq_copy(ph):
        return pltpu.make_async_copy(wq_hbm.at[:, pl.ds(hoff[ph] * DH, QH[ph] * DH)],
                                     wq_scr[ph].at[:, pl.ds(0, QH[ph] * DH)], wq_sem.at[ph])

    def k_copies(j):
        ks = pl.ds(koff[j], KS[j])
        cols = pl.ds(0, QH[0] * DH)
        return (pltpu.make_async_copy(x_hbm.at[:, ks], x_scr.at[:, ks], x_sem.at[j]),
                pltpu.make_async_copy(wq_hbm.at[ks, cols], wq_scr[0].at[ks, cols], wk_sem.at[j]))

    def q_store(q_all, hh, he):
        q_all = (q_all * scale).astype(bf16)
        for bb in range(B):
            for h in range(hh, he):
                qo_scr[bb * Hkv + h // rep, (h % rep) * Sq:(h % rep + 1) * Sq, :] = (
                    q_all[bb * Sq:(bb + 1) * Sq, (h - hh) * DH:(h - hh + 1) * DH])

    def qproj(ph):
        h0, h1 = hoff[ph], hoff[ph + 1]
        for hh in range(h0, h1, rep):
            he = min(hh + rep, h1)
            q_store(jnp.dot(x_scr[...], wq_scr[ph][:, (hh - h0) * DH:(he - h0) * DH],
                            preferred_element_type=f32), hh, he)

    for j in range(len(KS)):
        for c in k_copies(j):
            c.start()
    st_scr[2 * R0:2 * NB] = jnp.ones((2 * (NB - R0),) + st_scr.shape[1:], f32)
    z0 = jax.lax.fori_loop(0, 2, lambda i, c: jax.lax.shift_right_logical(i, 10), jnp.int32(0))
    for j in range(len(KS)):
        for c in k_copies(j):
            c.wait()
        if j == 0:
            wq_copy(1).start(priority=1)
        if j == len(KS) - 1:
            wq_copy(2).start(priority=1)
        part = jnp.dot(x_scr[:, koff[j]:koff[j + 1]], wq_scr[0][koff[j]:koff[j + 1], 0:QH[0] * DH],
                       preferred_element_type=f32)
        if j > 0:
            part = part + qa_scr[...]
        if j < len(KS) - 1:
            qa_scr[...] = part
        else:
            q_store(part, 0, QH[0])
    wq_copy(1).wait()
    wq_copy(3).start(priority=1)
    kv_start(0, 1, R0)
    qproj(1)
    wq_copy(2).wait()
    kv_start(R0, 0)
    qproj(2)

    def finalize(pair, i, z):
        l = jnp.sum(st_scr[2 * i + z], axis=-1, keepdims=True)
        r0 = pl.reciprocal(l, approx=True)
        inv = r0 * (2.0 - l * r0)
        qo_scr[pair] = (st_scr[2 * i + 1 + z] * inv).astype(bf16)

    def attend(pair0, slot, n, prev, z):
        for i in range(n):
            for c in range(nc):
                if c == FINC and prev is not None:
                    finalize(prev + i, i, z)
                s = jax.lax.dot_general(qo_scr[pair0 + i], k_buf[slot, i, c * CH:(c + 1) * CH, :],
                                        _NT, preferred_element_type=f32)
                mp = None if c == 0 else m_scr[(c - 1) % 2][z]
                for tt in range(CH // 128):
                    st = s[:, tt * 128:(tt + 1) * 128]
                    mp = st if mp is None else jnp.maximum(mp, st)
                if c < nc - 1:
                    s_scr[c] = s
                    m_scr[c % 2][0] = mp
                else:
                    sl_scr[0] = s
            m = jnp.max(mp, axis=-1, keepdims=True)
            lp = None
            acc = None
            last = i == n - 1

            def ex(c):
                nonlocal lp
                p = jnp.exp2((s_scr[c + z] if c < nc - 1 else sl_scr[z]) - m)
                for tt in range(CH // 128):
                    pt = p[:, tt * 128:(tt + 1) * 128]
                    lp = pt if lp is None else lp + pt
                return p.astype(bf16)

            for c in range(nc - 1 if last else nc):
                oc = jnp.dot(ex(c), v_buf[slot, i, c * CH:(c + 1) * CH, :],
                             preferred_element_type=f32)
                acc = oc if acc is None else acc + oc
                if c + 1 < nc - 1:
                    s_scr[nc - 1, 0:8, 0:128] = oc[TROW - 8:TROW]
                elif c + 1 < nc and not last:
                    sl_scr[1, 0:8, 0:128] = oc[TROW - 8:TROW]
                if last and c == 0:
                    sl_scr[1, 0:8, 0:128] = oc[0:8]
                    pt_scr[0] = ex(nc - 1)
                    vt_scr[0] = v_buf[slot, i, (nc - 1) * CH:nc * CH, :]
            st_scr[2 * i] = lp
            st_scr[2 * i + 1] = acc

    def pv_tail(i, z):
        st_scr[2 * i + 1] = st_scr[2 * i + 1] + jnp.dot(pt_scr[z], vt_scr[z],
                                                        preferred_element_type=f32)

    wq_copy(3).wait()
    kv_wait(0, 1, R0)
    qproj(3)
    attend(0, 1, R0, None, z0)
    kv_start(R0 + NB, 1)

    def step(t, carry):
        slot = jnp.bitwise_and(t, 1)
        pair0 = R0 + t * NB
        kv_wait(pair0, slot)
        z = jax.lax.shift_right_logical(t, 10)
        pv_tail(jnp.where(t > 0, NB - 1, R0 - 1), z)
        attend(pair0, slot, NB, jnp.maximum(pair0 - NB, 0), z)

        @pl.when(t + 2 < nsteps)
        def _():
            kv_start(pair0 + 2 * NB, slot)

        @pl.when(t < NWO)
        def _():
            rows = pl.ds(pl.multiple_of(t * (HQ * DH // NWO), 16), HQ * DH // NWO)
            pltpu.make_async_copy(wo_hbm.at[rows], wo_scr.at[rows], wo_sem).start(priority=1)
        return carry

    jax.lax.fori_loop(0, nsteps, step, 0)

    pltpu.make_async_copy(wo_hbm, wo_scr, wo_sem).wait()
    pv_tail(NB - 1, z0)
    NW = D // OSPLIT
    RQ = B * Sq // LSPLIT

    def out_copy(n, rq=None):
        cols = pl.ds(n * NW, NW)
        if rq is None:
            return pltpu.make_async_copy(out_scr.at[:, cols], out_hbm.at[:, cols], out_sem.at[n])
        rows = pl.ds(rq * RQ, RQ)
        return pltpu.make_async_copy(out_scr.at[rows, cols], out_hbm.at[rows, cols],
                                     out_sem.at[n + rq])

    for n in range(OSPLIT):
        acc = None
        for g in range(Hkv):
            if n == 0 and g == FING:
                for i in range(NB):
                    finalize(npairs - NB + i, i, 0)
            o_g = jnp.concatenate(
                [jnp.concatenate([qo_scr[bb * Hkv + g, r * Sq:(r + 1) * Sq, :] for r in range(rep)],
                                 axis=1)
                 for bb in range(B)], axis=0)
            c = jnp.dot(o_g, wo_scr[g * GW:(g + 1) * GW, n * NW:(n + 1) * NW],
                        preferred_element_type=f32)
            acc = c if acc is None else acc + c
        if n < OSPLIT - 1:
            out_scr[:, n * NW:(n + 1) * NW] = acc.astype(bf16)
            out_copy(n).start()
        else:
            for rq in range(LSPLIT):
                out_scr[rq * RQ:(rq + 1) * RQ, n * NW:(n + 1) * NW] = (
                    acc[rq * RQ:(rq + 1) * RQ].astype(bf16))
                out_copy(n, rq).start()
    for n in range(OSPLIT - 1):
        out_copy(n).wait()
    for rq in range(LSPLIT):
        out_copy(OSPLIT - 1, rq).wait()


@jax.jit
def pallas_standalone__gqa_block_cached__near_ridge_kernel(x, k_cache, v_cache, wq, wo):
    B, Sq, D = x.shape
    _, Hkv, Sk, Dh = k_cache.shape
    rep = HQ // Hkv
    M = rep * Sq
    npairs = B * Hkv
    assert Dh == DH and sum(QH) == HQ and sum(KS) == D and Sk % CH == 0 and Sk // CH > FINC
    assert (npairs - R0) % NB == 0 and (npairs - R0) // NB >= max(NWO, 2)
    assert 0 < NB - R0 <= R0
    assert (npairs - NB) % Hkv >= FING and NB <= Hkv - FING
    assert 8 <= TROW <= M and Sk // CH >= 3
    scale = (Dh ** -0.5) * math.log2(math.e)
    kern = functools.partial(_kernel, B=B, Sq=Sq, Sk=Sk, D=D, rep=rep, Hkv=Hkv, scale=scale)
    bf = jnp.bfloat16
    f32 = jnp.float32
    opts = dict(vmem_limit_bytes=110 * 1024 * 1024, disable_bounds_checks=True)
    try:
        params = pltpu.CompilerParams(disable_semaphore_checks=True, **opts)
    except TypeError:
        params = pltpu.CompilerParams(**opts)
    out = pl.pallas_call(
        kern,
        in_specs=[pl.BlockSpec(memory_space=pl.ANY)] * 5,
        out_specs=pl.BlockSpec(memory_space=pl.ANY),
        out_shape=jax.ShapeDtypeStruct((B * Sq, D), x.dtype),
        scratch_shapes=[
            pltpu.VMEM((B * Sq, D), bf),
            *[pltpu.VMEM((D, (n + 1) * Dh), bf) for n in QH],
            pltpu.VMEM((HQ * Dh, D), bf),
            pltpu.VMEM((2, NB, Sk, Dh), bf),
            pltpu.VMEM((2, NB, Sk, Dh), bf),
            pltpu.VMEM((npairs, M, Dh), bf),
            pltpu.VMEM((2 * NB, M, Dh), f32),
            pltpu.VMEM((B * Sq, D), bf),
            pltpu.VMEM((Sk // CH, M, CH), f32),
            pltpu.VMEM((2, M, CH), f32),
            pltpu.VMEM((1, M, 128), f32),
            pltpu.VMEM((1, M, 128), f32),
            pltpu.VMEM((1, M, CH), bf),
            pltpu.VMEM((1, CH, Dh), bf),
            pltpu.VMEM((B * Sq, QH[0] * Dh), f32),
            pltpu.SemaphoreType.DMA((len(KS),)),
            pltpu.SemaphoreType.DMA((len(KS),)),
            pltpu.SemaphoreType.DMA((len(QH),)),
            pltpu.SemaphoreType.DMA(()),
            pltpu.SemaphoreType.DMA((2,)),
            pltpu.SemaphoreType.DMA((2,)),
            pltpu.SemaphoreType.DMA((OSPLIT - 1 + LSPLIT,)),
        ],
        compiler_params=params,
    )(x.reshape(B * Sq, D), k_cache.reshape(npairs, Sk, Dh), v_cache.reshape(npairs, Sk, Dh), wq, wo)
    return out.reshape(B, Sq, D)
```
